```python
import jax
import jax.numpy as jnp

def _softmax(x, axis=-1):
    return jax.nn.softmax(x, axis=axis)
def _gelu(x):
    return jax.nn.gelu(x, approximate=True)
def _silu(x):
    return jax.nn.silu(x)
def _sigmoid(x):
    return jax.nn.sigmoid(x)
def _layernorm(x, axis=-1, eps=1e-5):
    m = jnp.mean(x, axis=axis, keepdims=True)
    v = jnp.var(x, axis=axis, keepdims=True)
    return (x - m) / jnp.sqrt(v + eps)
def _scatter_add(tgt, idx, src, axis=0):
    return tgt.at[idx].add(src)
def _segment_sum(src, seg, n):
    return jax.ops.segment_sum(src, seg, n)
class _Rng:
    def __init__(self, key):
        self._k = key
    def _next(self):
        self._k, sub = jax.random.split(self._k)
        return sub
    def normal(self, shape):
        return jax.random.normal(self._next(), shape, dtype=jnp.bfloat16)
    def randint(self, lo, hi, shape):
        return jax.random.randint(self._next(), shape, lo, hi, dtype=jnp.int32)
    def uniform(self, shape, lo=0.0, hi=1.0):
        return jax.random.uniform(self._next(), shape, jnp.bfloat16, lo, hi)
    def permutation(self, n):
        return jax.random.permutation(self._next(), n)


kernel_name = 'concat_heads__gqa_block_cached__gqa_block_cached__near_ridge'

def _fwd_setup_inputs():
    _rng = _Rng(jax.random.key(int.from_bytes(__import__("os").urandom(4), "little")))
    _w = (lambda a: (lambda t: t.astype(jnp.bfloat16) if jnp.issubdtype(t.dtype, jnp.floating) else t)(jnp.asarray(a)))
    def _A_setup():
        B, Sq, D = 16, 112, 640
        Hq, Hkv, Sk, Dh = 32, 32, 512, 128
        assert Hq % Hkv == 0, (Hq, Hkv)
        return {
            "x": _w((lambda *s: _rng.normal(s) * 0.05)(B, Sq, D)),
            "k_cache": _w((lambda *s: _rng.normal(s) * 0.05)(B, Hkv, Sk, Dh)),
            "v_cache": _w((lambda *s: _rng.normal(s) * 0.05)(B, Hkv, Sk, Dh)),
            "wq": _w((lambda *s: _rng.normal(s) * 0.05)(D, Hq * Dh) * (D ** -0.5)),
            "wo": _w((lambda *s: _rng.normal(s) * 0.05)(Hq * Dh, D) * ((Hq * Dh) ** -0.5)),
        }
    _A_in = _A_setup()

    def _B_setup():
        B, Sq, D = 16, 112, 640
        Hq, Hkv, Sk, Dh = 32, 32, 512, 128
        assert Hq % Hkv == 0, (Hq, Hkv)
        return {
            "x": _w((lambda *s: _rng.normal(s) * 0.05)(B, Sq, D)),
            "k_cache": _w((lambda *s: _rng.normal(s) * 0.05)(B, Hkv, Sk, Dh)),
            "v_cache": _w((lambda *s: _rng.normal(s) * 0.05)(B, Hkv, Sk, Dh)),
            "wq": _w((lambda *s: _rng.normal(s) * 0.05)(D, Hq * Dh) * (D ** -0.5)),
            "wo": _w((lambda *s: _rng.normal(s) * 0.05)(Hq * Dh, D) * ((Hq * Dh) ** -0.5)),
        }
    _B_in = _B_setup()

    return {
        "A_x": _A_in["x"],
        "A_k_cache": _A_in["k_cache"],
        "A_v_cache": _A_in["v_cache"],
        "A_wq": _A_in["wq"],
        "A_wo": _A_in["wo"],
        "B_x": _B_in["x"],
        "B_k_cache": _B_in["k_cache"],
        "B_v_cache": _B_in["v_cache"],
        "B_wq": _B_in["wq"],
        "B_wo": _B_in["wo"],
    }

def _fwd_reference(A_x, A_k_cache, A_v_cache, A_wq, A_wo, B_x, B_k_cache, B_v_cache, B_wq, B_wo):
    def _A_ref(x, k_cache, v_cache, wq, wo):
        B, Sq, D = x.shape
        Hq, Dh = 32, 128
        Hkv = k_cache.shape[1]
        rep = Hq // Hkv
        q = (lambda x, *d: x.transpose(*d))((x @ wq).reshape(B, Sq, Hq, Dh), 0, 2, 1, 3)
        k = jnp.repeat(k_cache, rep, axis=1)
        v = jnp.repeat(v_cache, rep, axis=1)
        scores = jnp.einsum("bhqd,bhkd->bhqk", q, k) * (Dh ** -0.5)
        p = _softmax(scores, axis=-1)
        o = jnp.einsum("bhqk,bhkd->bhqd", p, v)
        return (lambda x, *d: x.transpose(*d))(o, 0, 2, 1, 3).reshape(B, Sq, Hq * Dh) @ wo

    def _B_ref(x, k_cache, v_cache, wq, wo):
        B, Sq, D = x.shape
        Hq, Dh = 32, 128
        Hkv = k_cache.shape[1]
        rep = Hq // Hkv
        q = (lambda x, *d: x.transpose(*d))((x @ wq).reshape(B, Sq, Hq, Dh), 0, 2, 1, 3)
        k = jnp.repeat(k_cache, rep, axis=1)
        v = jnp.repeat(v_cache, rep, axis=1)
        scores = jnp.einsum("bhqd,bhkd->bhqk", q, k) * (Dh ** -0.5)
        p = _softmax(scores, axis=-1)
        o = jnp.einsum("bhqk,bhkd->bhqd", p, v)
        return (lambda x, *d: x.transpose(*d))(o, 0, 2, 1, 3).reshape(B, Sq, Hq * Dh) @ wo

    a = _A_ref(A_x, A_k_cache, A_v_cache, A_wq, A_wo)
    b = _B_ref(B_x, B_k_cache, B_v_cache, B_wq, B_wo)
    return jnp.concatenate([a, b], axis=-1)


def setup_inputs():
    _inp = _fwd_setup_inputs()
    _gk = jax.random.fold_in(jax.random.key(int.from_bytes(__import__("os").urandom(4), "little")), 2**31 - 1)
    _shapes = [[16, 112, 1280]]
    _dtypes = ['bfloat16']
    _gks = jax.random.split(_gk, len(_shapes))
    _gs = [jax.random.normal(k, s, dtype=jnp.dtype(d)) * 0.05 for k, s, d in zip(_gks, _shapes, _dtypes)]
    _inp["grad_out"] = _gs[0]
    return _inp

def reference(A_x, A_k_cache, A_v_cache, A_wq, A_wo, B_x, B_k_cache, B_v_cache, B_wq, B_wo, grad_out):
    _const = dict()
    def _f(*_d):
        return _fwd_reference(**{'A_x': _d[0], 'A_k_cache': _d[1], 'A_v_cache': _d[2], 'A_wq': _d[3], 'A_wo': _d[4], 'B_x': _d[5], 'B_k_cache': _d[6], 'B_v_cache': _d[7], 'B_wq': _d[8], 'B_wo': _d[9], **_const})
    _out, _vjp = jax.vjp(_f, A_x, A_k_cache, A_v_cache, A_wq, A_wo, B_x, B_k_cache, B_v_cache, B_wq, B_wo)
    _grads = _vjp(grad_out)
    _out0 = jnp.asarray(_out)
    return (_out0, *[jnp.asarray(_g) for _g in _grads])
```

```python
import math
import jax
import jax.numpy as jnp
from jax import lax
import jax.experimental.pallas as pl
import jax.experimental.pallas.tpu as pltpu

F32 = jnp.float32
BF16 = jnp.bfloat16
NT = (((1,), (1,)), ((), ()))
TN = (((0,), (0,)), ((), ()))

B, SQ, D, H, SK, DH = 16, 112, 640, 32, 512, 128
M = B * SQ
HP = 2
W = HP * DH
SPB = H // HP
NSTEP = 2 * SPB
SCALE = DH ** -0.5
LOG2E = math.log2(math.e)
MC = 448


def _dot(a, b, dn=None):
    if dn is None:
        return jnp.dot(a, b, preferred_element_type=F32)
    return lax.dot_general(a, b, dn, preferred_element_type=F32)


def _stage1(q, do, k, v):
    s = _dot((q * (SCALE * LOG2E)).astype(BF16), k, NT)
    dp = _dot(do.astype(BF16), v, NT)
    m = jnp.max(s, axis=1, keepdims=True)
    e = jnp.exp2(s - m)
    l = jnp.sum(e, axis=1, keepdims=True)
    r = pl.reciprocal(l, approx=False, full_range=False)
    t = e * dp
    dd = jnp.sum(t, axis=1, keepdims=True) * r
    ds = t - e * dd
    rs = r * SCALE
    return (e.astype(BF16), ds.astype(BF16), (do * r).astype(BF16),
            (q * rs).astype(BF16), r, rs)


def _kernel(ax, ak, av, awq, awo, bx, bk, bv, bwq, bwo, g_hbm,
            out_hbm, dax, dak, dav, dawq, dawo, dbx, dbk, dbv, dbwq, dbwo,
            xbuf, gbuf, xT, gT, kbuf, vbuf, dkbuf, dvbuf,
            wqbuf, wobuf, dwqbuf, dwobuf, outacc, dxacc, outst, dxst,
            qs, dos, os_, dqs, sem_in, sem_out, sem_xg, sem_fin):
    ins = ((ak, av, awq, awo), (bk, bv, bwq, bwo))
    outs = ((dak, dav, dawq, dawo), (dbk, dbv, dbwq, dbwo))

    def in_copies(blk, hp, slot):
        k, v, wq, wo = ins[blk]
        h0 = hp * HP
        c0 = pl.multiple_of(hp * W, W)
        return (
            pltpu.make_async_copy(wq.at[:, pl.ds(c0, W)], wqbuf.at[slot], sem_in.at[slot * 4 + 2]),
            pltpu.make_async_copy(wo.at[pl.ds(c0, W), :], wobuf.at[slot], sem_in.at[slot * 4 + 3]),
            pltpu.make_async_copy(k.at[:, pl.ds(h0, HP)], kbuf.at[slot], sem_in.at[slot * 4]),
            pltpu.make_async_copy(v.at[:, pl.ds(h0, HP)], vbuf.at[slot], sem_in.at[slot * 4 + 1]),
        )

    def out_copies(blk, hp, slot):
        dk, dv, dwq, dwo = outs[blk]
        h0 = hp * HP
        c0 = pl.multiple_of(hp * W, W)
        return (
            pltpu.make_async_copy(dkbuf.at[slot], dk.at[:, pl.ds(h0, HP)], sem_out.at[slot * 4]),
            pltpu.make_async_copy(dvbuf.at[slot], dv.at[:, pl.ds(h0, HP)], sem_out.at[slot * 4 + 1]),
            pltpu.make_async_copy(dwqbuf.at[slot], dwq.at[:, pl.ds(c0, W)], sem_out.at[slot * 4 + 2]),
            pltpu.make_async_copy(dwobuf.at[slot], dwo.at[pl.ds(c0, W), :], sem_out.at[slot * 4 + 3]),
        )

    def xg_copies(blk):
        return (
            pltpu.make_async_copy((ax, bx)[blk], xbuf.at[blk], sem_xg.at[2 * blk]),
            pltpu.make_async_copy(g_hbm.at[:, pl.ds(blk * D, D)], gbuf.at[blk], sem_xg.at[2 * blk + 1]),
        )

    def fin_copies(blk):
        return (
            pltpu.make_async_copy(outst, out_hbm.at[:, pl.ds(blk * D, D)], sem_fin.at[0]),
            pltpu.make_async_copy(dxst, (dax, dbx)[blk], sem_fin.at[1]),
        )

    for c in xg_copies(0):
        c.start()
    for c in in_copies(0, 0, 0):
        c.start()

    def step(t, carry):
        slot = t % 2
        blk = t // SPB
        hp = t % SPB

        for bb in range(2):
            @pl.when(t == bb * SPB)
            def _():
                for c in xg_copies(bb):
                    c.wait()
                for c in range(M // 128):
                    r = slice(c * 128, (c + 1) * 128)
                    xT[:, r] = xbuf[bb, r, :].T
                    gT[:, r] = gbuf[bb, r, :].T
                outacc[...] = jnp.zeros(outacc.shape, F32)
                dxacc[...] = jnp.zeros(dxacc.shape, F32)

        for c in in_copies(0, 0, slot):
            c.wait()

        @pl.when(t == 1)
        def _():
            for c in xg_copies(1):
                c.start()

        nt = t + 1
        for bb in range(2):
            @pl.when(jnp.logical_and(nt // SPB == bb, nt < NSTEP))
            def _():
                for c in in_copies(bb, nt % SPB, 1 - slot):
                    c.start()

        @pl.when(t >= 2)
        def _():
            for c in out_copies(0, 0, slot):
                c.wait()

        x = xbuf.at[blk]
        g = gbuf.at[blk]
        wq = wqbuf.at[slot]
        wo = wobuf.at[slot]
        for hh in range(HP):
            cs = slice(hh * DH, (hh + 1) * DH)
            for c in range(M // MC):
                r = slice(c * MC, (c + 1) * MC)
                qs[r, cs] = _dot(x[r, :], wq[:, cs])
            for c in range(M // MC):
                r = slice(c * MC, (c + 1) * MC)
                dos[r, cs] = _dot(g[r, :], wo[cs, :], NT)

        prev = None
        seq = [(hh, b) for hh in range(HP) for b in range(B)]
        for i in range(len(seq) + 1):
            if i < len(seq):
                hh, b = seq[i]
                cs = slice(hh * DH, (hh + 1) * DH)
                rows = slice(b * SQ, (b + 1) * SQ)
                cur = _stage1(qs[rows, cs], dos[rows, cs], kbuf[slot, b, hh], vbuf[slot, b, hh])
            if prev is not None:
                hh, b = seq[i - 1]
                cs = slice(hh * DH, (hh + 1) * DH)
                rows = slice(b * SQ, (b + 1) * SQ)
                eb, dsb, dor, qr, r, rs = prev
                os_[rows, cs] = (_dot(eb, vbuf[slot, b, hh]) * r).astype(BF16)
                dqs[rows, cs] = (_dot(dsb, kbuf[slot, b, hh]) * rs).astype(BF16)
                for j in range(4):
                    js = slice(j * 128, (j + 1) * 128)
                    dvbuf[slot, b, hh, js, :] = _dot(eb[:, js], dor, TN).astype(BF16)
                for j in range(4):
                    js = slice(j * 128, (j + 1) * 128)
                    dkbuf[slot, b, hh, js, :] = _dot(dsb[:, js], qr, TN).astype(BF16)
            prev = cur

        for hh in range(HP):
            cs = slice(hh * DH, (hh + 1) * DH)
            dwobuf[slot, cs, :] = _dot(gT[...], os_[:, cs]).astype(BF16).T
            dwqbuf[slot, :, cs] = _dot(xT[...], dqs[:, cs]).astype(BF16)
        for c in range(M // MC):
            r = slice(c * MC, (c + 1) * MC)
            outacc[r, :] += _dot(os_[r, :], wo[...])
        for c in range(M // MC):
            r = slice(c * MC, (c + 1) * MC)
            dxacc[r, :] += _dot(dqs[r, :], wq[...], NT)

        for bb in range(2):
            @pl.when(blk == bb)
            def _():
                for c in out_copies(bb, hp, slot):
                    c.start()

        for bb in range(2):
            @pl.when(t == bb * SPB + SPB - 1)
            def _():
                if bb == 1:
                    for c in fin_copies(0):
                        c.wait()
                outst[...] = outacc[...].astype(BF16)
                dxst[...] = dxacc[...].astype(BF16)
                for c in fin_copies(bb):
                    c.start()
        return carry

    lax.fori_loop(0, NSTEP, step, 0)
    for slot in range(2):
        for c in out_copies(0, 0, slot):
            c.wait()
    for c in fin_copies(1):
        c.wait()


@jax.jit
def pallas_concat_heads__gqa_block_cached__gqa_block_cached__near_ridge_kernel(
    A_x, A_k_cache, A_v_cache, A_wq, A_wo, B_x, B_k_cache, B_v_cache, B_wq, B_wo, grad_out,
):
    S = jax.ShapeDtypeStruct
    one = [S((M, D), BF16), S((B, H, SK, DH), BF16), S((B, H, SK, DH), BF16),
           S((D, H * DH), BF16), S((H * DH, D), BF16)]
    any_spec = pl.BlockSpec(memory_space=pl.ANY)
    V = pltpu.VMEM
    res = pl.pallas_call(
        _kernel,
        out_shape=[S((M, 2 * D), BF16)] + one + one,
        in_specs=[any_spec] * 11,
        out_specs=[any_spec] * 11,
        scratch_shapes=[
            V((2, M, D), BF16), V((2, M, D), BF16), V((D, M), BF16), V((D, M), BF16),
            V((2, B, HP, SK, DH), BF16), V((2, B, HP, SK, DH), BF16),
            V((2, B, HP, SK, DH), BF16), V((2, B, HP, SK, DH), BF16),
            V((2, D, W), BF16), V((2, W, D), BF16), V((2, D, W), BF16), V((2, W, D), BF16),
            V((M, D), F32), V((M, D), F32), V((M, D), BF16), V((M, D), BF16),
            V((M, W), F32), V((M, W), F32), V((M, W), BF16), V((M, W), BF16),
            pltpu.SemaphoreType.DMA((8,)), pltpu.SemaphoreType.DMA((8,)),
            pltpu.SemaphoreType.DMA((4,)), pltpu.SemaphoreType.DMA((2,)),
        ],
        compiler_params=pltpu.CompilerParams(vmem_limit_bytes=100 * 1024 * 1024),
        name="attn_fwdbwd",
    )(A_x.reshape(M, D), A_k_cache, A_v_cache, A_wq, A_wo,
      B_x.reshape(M, D), B_k_cache, B_v_cache, B_wq, B_wo, grad_out.reshape(M, 2 * D))
    out = res[0].reshape(B, SQ, 2 * D)
    return (out, res[1].reshape(B, SQ, D), res[2], res[3], res[4], res[5],
            res[6].reshape(B, SQ, D), res[7], res[8], res[9], res[10])
```

```python
import functools
import math
import jax
import jax.numpy as jnp
from jax import lax
import jax.experimental.pallas as pl
import jax.experimental.pallas.tpu as pltpu

F32 = jnp.float32
BF16 = jnp.bfloat16
NT = (((1,), (1,)), ((), ()))
TN = (((0,), (0,)), ((), ()))

B, SQ, D, H, SK, DH = 16, 112, 640, 32, 512, 128
M = B * SQ
HP = 2
W = HP * DH
SPB = H // HP
NSTEP = 2 * SPB
SCALE = DH ** -0.5
LOG2E = math.log2(math.e)
MC = 448
T = 128


_SCHEME = (
    "+00 +00-02-10+12 +00+04-22+32+60",
    "+00+01 -10+12 +01+02+04",
    "+10-40 +01 +11+13-14-61",
    "+11-41 +11 +12-41",
    "+30 +00-10 +10-20-22+30+32+34",
    "+01-61 +10 +00+02+04+40",
    "+50 +04 -23+24-32+50-53+54+64",
    "+51 +14 +23-32+34+44-51-52+54",
    "+40 +03-13 -03+11+13-14-40+41+43-44-63",
    "+40+41 +13 +03+12+23+42+43+53",
    "+20+21 +01 -20+21+51",
    "+21 -01+11 +01+21+23-24-31-33",
    "+60+61 +02 +03-12+32+52+62+63",
    "+61 -02+12 +00+02+04-12-42+60+61+62-64",
    "+00+21 +01+10-12 +01-22",
    "-00+20 -00-01+02 +22",
    "+01-21 +10+11-12 +01",
    "-30-31+51 +00-04-10 +32+34-50",
    "+31-51 +00-04-10+14 -04+34",
    "+30+31-50-51 -00+04 +50",
    "-20-21+50 +01-11-14 -23+24+51",
    "+20-50 +01+04-11-14 -14+24",
    "-20-21+50+51 +11+14 +51",
    "+21-30 +01+10 +20+22-31-33",
    "+20+30 +00+01 +20+22",
    "+21+31 +10+11 +31+33",
    "+11+40 -01+03-13 -11-13+14-41",
    "+10+11 -01+03 +10+13-14",
    "+11 -01+03+11-13 +11-14+23-33+41",
    "+40+41-51 +03+04-13 +23+44+53",
    "+10+20-50 +03+04 +14",
    "-41+51 +03+04-13-14 +44",
    "-40+61 -02+13 +03+12+42+63",
    "+41+61 +12-13 +12+42",
    "+40+60 -02+03 +03+63",
    "-50+60+61 -02+12+14 +32+52+64",
    "+50+51-60-61 +12+14 +32+52",
    "+50-60 -02-04+12+14 +64",
    "+00+61 +02+10-12 +00+02+04+60",
    "-00+60 +00 +03+60",
    "+30+31 +10 +30-31+50",
    "-01+40+41+61 +00+03-13 +03+40",
    "+01-41-61 +00+03-10-13 +40",
    "+00+01-40-41-60-61 +00+03 +03",
    "-10+40-60-61 -02-11+12 +12+61",
    "+10-40+60 +01-02-11+12 +61",
    "+10+11-40-41+60+61 -11+12 +12",
    "+11+30 +01-03+10 +10-33",
    "-10+30 -00-01+03 +10",
    "+11-31 +10+11-13 +33",
    "-00+31-51 +00-04-10+12 +04+32",
    "-01-31+51 +12-14 +04",
    "+00+30-50 +02-04 +32",
    "+11-20+50 -01+03+11+14 +14-23",
    "+11+21-51 +13+14 +23",
    "-40-41+50+51 +03+04 +23+53",
)
MB = 2 * T


def _plan():
    def form(txt):
        return {(int(txt[i + 1]), int(txt[i + 2])): 1 if txt[i] == "+" else -1 for i in range(0, len(txt), 3)}

    alg = [tuple(form(f) for f in row.split()) for row in _SCHEME]
    for a in [(i, l) for i in range(M // MB) for l in range(HP)]:
        for b in [(l, j) for l in range(HP) for j in range(D // T)]:
            got = {}
            for u, v, w in alg:
                for c, x in w.items():
                    got[c] = got.get(c, 0) + x * u.get(a, 0) * v.get(b, 0)
            want = {(a[0], b[1]): 1} if a[1] == b[0] else {}
            assert {c: x for c, x in got.items() if x} == want
    alg.sort(key=lambda t: not any(i == 0 for i, _ in t[0]))
    return [dict(off=n * MB, mb=MB,
                 u=[(s, i * MB, j) for (i, j), s in u.items()],
                 v=[(s, j, c) for (j, c), s in v.items()],
                 w=[(s, i * MB, c) for (i, c), s in w.items()],
                 um=[(s, i * MB, 2 if u.get((i, 1 - j)) == s else j) for (i, j), s in u.items()
                     if j == 0 or u.get((i, 0)) != s],
                 vm=[(s, 2 if v.get((1 - j, c)) == -s else j, c) for (j, c), s in v.items()
                     if j == 0 or v.get((0, c)) != -s])
            for n, (u, v, w) in enumerate(alg)]


PRODS = _plan()
NP = len(PRODS)
PR = NP * MB
PRA = (NP - 8) * MB
PIN = 3
LAG = 4
TAIL = 4
ST = 16
ROWBLK = [(i * MB, MB) for i in range(M // MB)]


def _dot(a, b, dn=None):
    if dn is None:
        return jnp.dot(a, b, preferred_element_type=F32)
    return lax.dot_general(a, b, dn, preferred_element_type=F32)


def _comb(signs, vals):
    order = sorted(range(len(signs)), key=lambda i: -signs[i])
    acc = vals[order[0]] if signs[order[0]] > 0 else -vals[order[0]]
    for i in order[1:]:
        acc = acc + vals[i] if signs[i] > 0 else acc - vals[i]
    return acc


def _tile(i):
    return slice(i * T, (i + 1) * T)


def _stage1(q, do, k, v):
    s = _dot((q * (SCALE * LOG2E)).astype(BF16), k, NT)
    dp = _dot(do.astype(BF16), v, NT)
    m = jnp.max(s, axis=1, keepdims=True)
    e = jnp.exp2(s - m)
    l = jnp.sum(e, axis=1, keepdims=True)
    r = pl.reciprocal(l, approx=False, full_range=False)
    t = e * dp
    dd = jnp.sum(t, axis=1, keepdims=True) * r
    ds = t - e * dd
    rs = r * SCALE
    return (e.astype(BF16), [e[:, _tile(j)].astype(BF16) for j in range(SK // T)],
            ds.astype(BF16), [ds[:, _tile(j)].astype(BF16) for j in range(SK // T)],
            (do * r).astype(BF16), (q * rs).astype(BF16), r, rs)


def _kernel(ax, ak, av, awq, awo, bx, bk, bv, bwq, bwo, g_hbm,
            out_hbm, dax, dak, dav, dawq, dawo, dbx, dbk, dbv, dbwq, dbwo,
            xbuf, gbuf, gc, xc, gct, xct, kvbuf, dkvbuf,
            wqbuf, wobuf, dwqst, dwost, acc3, acc4, outst, dxst,
            p1a, p1b, p2a, p2b, os_, dqs, m5, m6, zr, sem_in, sem_out, sem_w, sem_xg, sem_fin):
    ins = ((ak, av, awq, awo), (bk, bv, bwq, bwo))
    outs = ((dak, dav, dawq, dawo), (dbk, dbv, dbwq, dbwo))
    copy = pltpu.make_async_copy

    def cols(hp):
        return pl.ds(hp * W if isinstance(hp, int) else pl.multiple_of(hp * W, W), W)

    def win_copies(blk, hp, slot):
        _, _, wq, wo = ins[blk]
        return [copy(wq.at[:, cols(hp)], wqbuf.at[slot], sem_in.at[slot * 4 + 2]),
                copy(wo.at[cols(hp), :], wobuf.at[slot], sem_in.at[slot * 4 + 3])]

    def kvin_copies(blk, hp, slot):
        k, v, _, _ = ins[blk]
        return [copy(k.at[:, pl.ds(hp * HP, HP)], kvbuf.at[slot, 0], sem_in.at[slot * 4]),
                copy(v.at[:, pl.ds(hp * HP, HP)], kvbuf.at[slot, 1], sem_in.at[slot * 4])]

    def kvin_wait(slot):
        copy(kvbuf.at[slot], kvbuf.at[slot], sem_in.at[slot * 4]).wait()

    def kv_copies(blk, hp, slot, hh):
        dk, dv, _, _ = outs[blk]
        h = hp * HP + hh
        return [copy(dkvbuf.at[slot, 0, pl.ds(0, B), hh], dk.at[:, h], sem_out.at[slot]),
                copy(dkvbuf.at[slot, 1, pl.ds(0, B), hh], dv.at[:, h], sem_out.at[slot])]

    def kv_wait(slot):
        buf = dkvbuf.at[slot, :, pl.ds(0, B)]
        copy(buf, buf, sem_out.at[slot]).wait()

    def w_copies(blk, hp, slot):
        _, _, dwq, dwo = outs[blk]
        return [copy(dwqst.at[slot], dwq.at[:, cols(hp)], sem_w.at[slot * 2]),
                copy(dwost.at[slot], dwo.at[cols(hp), :], sem_w.at[slot * 2 + 1])]

    def x_copy(blk):
        return copy((ax, bx)[blk], xbuf.at[blk], sem_xg.at[2 * blk])

    def g_copy(blk):
        return copy(g_hbm.at[:, pl.ds(blk * D, D)], gbuf.at[blk], sem_xg.at[2 * blk + 1])

    def fin_copies(blk):
        return [copy(outst, out_hbm.at[:, pl.ds(blk * D, D)], sem_fin.at[0]),
                copy(dxst, (dax, dbx)[blk], sem_fin.at[1])]

    def start(cs):
        for c in cs:
            c.start()

    def wait(cs):
        for c in cs:
            c.wait()

    def on_block(blk, valid, fn):
        if isinstance(blk, int):
            if valid:
                fn(blk)
            return
        for bb in range(2):
            pl.when(blk == bb if valid is True else jnp.logical_and(blk == bb, valid))(
                functools.partial(fn, bb))

    def w_forms(src, dst):
        blocks = {(r0, c): src(r0, c) for r0, _ in ROWBLK for c in range(D // T)}
        for p in PRODS:
            dst(p["off"], _comb([s for s, _, _ in p["w"]], [blocks[(r0, c)] for _, r0, c in p["w"]]).astype(BF16))

    def precompute(blk):
        for src, nat, trn in ((gbuf, gc, gct), (xbuf, xc, xct)):
            tiles = {(i, c): src[blk, _tile(i), _tile(c)].T.astype(F32)
                     for i in range(M // T) for c in range(D // T)}
            for hf in range(MB // T):
                for a in range(0, T, ST):
                    def store(o, val):
                        trn[o // T + hf, a:a + ST, :] = val
                    w_forms(lambda r0, c: tiles[(r0 // T + hf, c)][a:a + ST], store)
            for a in range(0, MB, ST):
                def store(o, val):
                    nat[o + a:o + a + ST, :] = val
                w_forms(lambda r0, c: src[blk, r0 + a:r0 + a + ST, _tile(c)].astype(F32), store)

    def finalize(acc, st):
        for a in range(0, MB, ST):
            vals = {p["off"]: acc[p["off"] + a:p["off"] + a + ST, :] for p in PRODS}
            for r0, _ in ROWBLK:
                row = []
                for c in range(D // T):
                    ts = [(s, p["off"]) for p in PRODS for s, rr, cc in p["w"] if (rr, cc) == (r0, c)]
                    row.append(_comb([s for s, _ in ts], [vals[o] for _, o in ts]))
                st[r0 + a:r0 + a + ST, :] = jnp.concatenate(row, 1).astype(BF16)

    def w_comb(p, ref, tr):
        return _comb([s for s, _, _ in p["v"]],
                     [(ref[_tile(c), _tile(j)] if tr else ref[_tile(j), _tile(c)]).astype(F32)
                      for _, j, c in p["v"]]).astype(BF16)

    def u_comb(p, ref):
        u = _comb([s for s, _, _ in p["um"]], [ref[r0:r0 + MB, _tile(j)] for _, r0, j in p["um"]])
        return u.astype(BF16), [u[a:a + T].astype(BF16) for a in range(0, MB, T)]

    def in_proj(lhs, wref, tr, dsts, z):
        ws = {}
        for p in PRODS:
            o = p["off"]
            ref, a0 = (dsts[0], o) if o < PRA else (dsts[1], o - PRA)
            ws[o] = w_comb(p, wref, tr)
            ref[0, a0:a0 + MB, :] = _dot(lhs[o:o + MB, :], ws[o], None if tr else NT)

        def rows(b, hh):
            pieces = []
            for r0, mb in ROWBLK:
                lo, hi = max(b * SQ, r0), min((b + 1) * SQ, r0 + mb)
                if lo < hi:
                    ts = [(s, p["off"] + lo - r0) for p in PRODS for s, rr, j in p["u"] if (rr, j) == (r0, hh)]
                    pieces.append(_comb([s for s, _ in ts], [
                        dsts[0][z, o:o + hi - lo, :] if o < PRA else dsts[1][z, o - PRA:o - PRA + hi - lo, :]
                        for _, o in ts]))
            return pieces[0] if len(pieces) == 1 else jnp.concatenate(pieces, 0)
        return rows, ws

    def attention(slot, q_rows, do_rows, after):
        prev = None
        seq = [(hh, b) for hh in range(HP) for b in range(B)]
        for i in range(len(seq) + 1):
            if i < len(seq):
                hh, b = seq[i]
                cur = _stage1(q_rows(b, hh), do_rows(b, hh),
                              kvbuf[slot, 0, b, hh], kvbuf[slot, 1, b, hh])
            if prev is not None:
                hh, b = seq[i - 1]
                rows = slice(b * SQ, (b + 1) * SQ)
                ef, eb, dsf, dsb, dor, qr, r, rs = prev
                for ref, val in ((os_, _dot(ef, kvbuf[slot, 1, b, hh]) * r),
                                 (dqs, _dot(dsf, kvbuf[slot, 0, b, hh]) * rs)):
                    ref[0, rows, _tile(hh)] = val
                    if hh == 1:
                        ref[0, rows, _tile(2)] = val + ref[0, rows, _tile(0)]
                for j in range(SK // T):
                    dkvbuf[slot, 1, b, hh, _tile(j), :] = _dot(eb[j], dor, TN).astype(BF16)
                for j in range(SK // T):
                    dkvbuf[slot, 0, b, hh, _tile(j), :] = _dot(dsb[j], qr, TN).astype(BF16)
                after(i - 1)
            prev = cur

    def post(slot, z0, z1, first, wos, wqs):
        fams = ((os_, gct, m6, acc3, wos, False), (dqs, xct, m5, acc4, wqs, True))
        srt = sorted(PRODS, key=lambda p: 2 * len(p["um"]) + len(p["vm"]))
        mix = [srt[i // 2] if i % 2 else srt[NP - 1 - i // 2] for i in range(NP)]
        order = []
        for i in range(NP + LAG):
            if i < NP:
                order.append((mix[i], 0))
            if i >= LAG:
                order.append((mix[i - LAG], 1))
        left = {(f, c): sum(cc == c for p in PRODS for _, _, cc in p["vm"])
                for f in range(2) for c in range(D // T)}
        seen = set()
        late = []
        for n, (p, f) in enumerate(order):
            o = p["off"]
            act, ct, mm, acc, wref, tr = fams[f]
            uf, u = u_comb(p, act.at[z1])
            if n == PIN:
                dkvbuf[slot, 0, B + z0, 0, 0:T, :] = u[0]
                u[0] = dkvbuf[slot, 0, B + z1, 0, 0:T, :]
            wv = wref[o]
            prod = _dot(jnp.concatenate([ct[o // T + hf] for hf in range(MB // T)], 1), uf)
            for s, j, c in p["vm"]:
                i = j * (D // T) + c
                if (f, i) in seen:
                    mm[i] = mm[i] + prod if s > 0 else mm[i] - prod
                else:
                    mm[i] = prod if s > 0 else -prod
                seen.add((f, i))
                left[(f, c)] -= 1
                if left[(f, c)] == 0:
                    for jj in range(HP):
                        val = mm[jj * (D // T) + c]
                        if (f, 2 * (D // T) + c) in seen:
                            dm = mm[2 * (D // T) + c]
                            val = val - dm if jj else val + dm
                        if tr:
                            dwqst[slot, _tile(c), _tile(jj)] = val.astype(BF16)
                        else:
                            dwost[slot, _tile(jj), _tile(c)] = val.astype(BF16).T

            def accumulate(o=o, acc=acc, u=u, wv=wv, tr=tr):
                for hf in range(MB // T):
                    rr = slice(o + hf * T, o + (hf + 1) * T)
                    part = _dot(u[hf], wv, NT if tr else None)
                    acc[rr, :] = part if first is True else jnp.where(first, 0.0, acc[rr, :]) + part

            if n < len(order) - TAIL:
                accumulate()
            else:
                late.append(accumulate)
        for fn in late:
            fn()

    for i in range(2):
        zr[i] = 0
    start([x_copy(0), g_copy(0)])

    def step(t, carry):
        slot = t % 2
        blk = t // SPB
        hp = t % SPB
        z0 = zr[0]
        z1 = zr[1]

        @pl.when(hp == 0)
        def _():
            @pl.when(t > 0)
            def _():
                finalize(acc3, outst)
                finalize(acc4, dxst)
                start(fin_copies(0))

            on_block(blk, True, lambda bb: x_copy(bb).wait())

            @pl.when(t == 0)
            def _():
                start(win_copies(0, 0, 0) + kvin_copies(0, 0, 0))

            on_block(blk, True, lambda bb: g_copy(bb).wait())
            precompute(blk)

        wait(win_copies(0, 0, slot))
        kvin_wait(slot)

        @pl.when(t >= 2)
        def _():
            kv_wait(slot)
            wait(w_copies(0, 0, slot))

        q_rows, wqs = in_proj(xc, wqbuf.at[slot], True, (p1a, p1b), z0)
        do_rows, wos = in_proj(gc, wobuf.at[slot], False, (p2a, p2b), z0)

        @pl.when(t == 0)
        def _():
            start(win_copies(0, 1, 1) + kvin_copies(0, 1, 1))

        def after(i):
            if i % B == B - 1:
                on_block(blk, True, lambda bb: start(kv_copies(bb, hp, slot, i // B)))

        attention(slot, q_rows, do_rows, after)
        nt = t + 2
        on_block(nt // SPB, True, lambda bb: start(kvin_copies(bb, nt % SPB, slot)))
        post(slot, z0, z1, hp == 0, wos, wqs)
        on_block(nt // SPB, True, lambda bb: start(win_copies(bb, nt % SPB, slot)))
        on_block(blk, True, lambda bb: start(w_copies(bb, hp, slot)))

        @pl.when(t == 2)
        def _():
            start([x_copy(1), g_copy(1)])

        return carry

    lax.fori_loop(0, NSTEP, step, 0)
    wait(fin_copies(0))
    finalize(acc3, outst)
    finalize(acc4, dxst)
    start(fin_copies(1))
    for slot in range(2):
        kv_wait(slot)
        wait(w_copies(0, 0, slot))
    wait(fin_copies(1))


@jax.jit
def pallas_concat_heads__gqa_block_cached__gqa_block_cached__near_ridge_kernel(
    A_x, A_k_cache, A_v_cache, A_wq, A_wo, B_x, B_k_cache, B_v_cache, B_wq, B_wo, grad_out,
):
    S = jax.ShapeDtypeStruct
    one = [S((M, D), BF16), S((B, H, SK, DH), BF16), S((B, H, SK, DH), BF16),
           S((D, H * DH), BF16), S((H * DH, D), BF16)]
    any_spec = pl.BlockSpec(memory_space=pl.ANY)
    V = pltpu.VMEM
    kv = V((2, 2, B, HP, SK, DH), BF16)
    dkv = V((2, 2, B + 1, HP, SK, DH), BF16)
    res = pl.pallas_call(
        _kernel,
        out_shape=[S((M, 2 * D), BF16)] + one + one,
        in_specs=[any_spec] * 11,
        out_specs=[any_spec] * 11,
        scratch_shapes=[
            V((2, M, D), BF16), V((2, M, D), BF16),
            V((PR, T), BF16), V((PR, T), BF16), V((PR // T, T, T), BF16), V((PR // T, T, T), BF16),
            kv, dkv,
            V((2, D, W), BF16), V((2, W, D), BF16), V((2, D, W), BF16), V((2, W, D), BF16),
            V((PR, T), F32), V((PR, T), F32), V((M, D), BF16), V((M, D), BF16),
            V((1, PRA, T), F32), V((1, PR - PRA, T), F32), V((1, PRA, T), F32), V((1, PR - PRA, T), F32), V((1, M, 3 * T), F32), V((1, M, 3 * T), F32),
            V((15, T, T), F32), V((15, T, T), F32),
            pltpu.SMEM((2,), jnp.int32),
            pltpu.SemaphoreType.DMA((8,)), pltpu.SemaphoreType.DMA((2,)),
            pltpu.SemaphoreType.DMA((4,)), pltpu.SemaphoreType.DMA((4,)),
            pltpu.SemaphoreType.DMA((2,)),
        ],
        compiler_params=pltpu.CompilerParams(vmem_limit_bytes=112 * 1024 * 1024, disable_bounds_checks=True),
        name="attn_fwdbwd",
    )(A_x.reshape(M, D), A_k_cache, A_v_cache, A_wq, A_wo,
      B_x.reshape(M, D), B_k_cache, B_v_cache, B_wq, B_wo, grad_out.reshape(M, 2 * D))
    out = res[0].reshape(B, SQ, 2 * D)
    return (out, res[1].reshape(B, SQ, D), res[2], res[3], res[4], res[5],
            res[6].reshape(B, SQ, D), res[7], res[8], res[9], res[10])
```
